```python
import os as _os
_os.environ.setdefault("JAX_PLATFORMS", "cpu")
import jax
import jax.numpy as jnp

def _softmax(x, axis=-1):
    return jax.nn.softmax(x, axis=axis)
def _gelu(x):
    return jax.nn.gelu(x, approximate=True)
def _silu(x):
    return jax.nn.silu(x)
def _sigmoid(x):
    return jax.nn.sigmoid(x)
def _layernorm(x, axis=-1, eps=1e-5):
    m = jnp.mean(x, axis=axis, keepdims=True)
    v = jnp.var(x, axis=axis, keepdims=True)
    return (x - m) / jnp.sqrt(v + eps)
def _scatter_add(tgt, idx, src, axis=0):
    return tgt.at[idx].add(src)
def _segment_sum(src, seg, n):
    return jax.ops.segment_sum(src, seg, n)
class _Rng:
    def __init__(self, key):
        self._k = key
    def _next(self):
        self._k, sub = jax.random.split(self._k)
        return sub
    def normal(self, shape):
        return jax.random.normal(self._next(), shape, dtype=jnp.bfloat16)
    def randint(self, lo, hi, shape):
        return jax.random.randint(self._next(), shape, lo, hi, dtype=jnp.int32)
    def uniform(self, shape, lo=0.0, hi=1.0):
        return jax.random.uniform(self._next(), shape, jnp.bfloat16, lo, hi)
    def permutation(self, n):
        return jax.random.permutation(self._next(), n)


kernel_name = 'gated_mix__spectral_gfnet__dense_activation_silu__prompt'

def setup_inputs():
    _rng = _Rng(jax.random.key(int.from_bytes(__import__("os").urandom(4), "little")))
    _w = (lambda a: (lambda t: t.astype(jnp.bfloat16) if jnp.issubdtype(t.dtype, jnp.floating) else t)(jnp.asarray(a)))
    def _A_setup():
        B, S, D = 1, 2048, 512
        Df = D // 2 + 1
        return {
            "x": _w((lambda *s: _rng.normal(s) * 0.05)(B, S, D)),
            "w_r": _w((lambda *s: _rng.normal(s) * 0.05)(S, Df) * 0.02),
            "w_i": _w((lambda *s: _rng.normal(s) * 0.05)(S, Df) * 0.02),
        }
    _A_in = _A_setup()

    def _B_setup():
        B, S, D, F = 1, 2048, 512, 1376
        return {
            "x": _w((lambda *s: _rng.normal(s) * 0.05)(B, S, D)),
            "w1": _w((lambda *s: _rng.normal(s) * 0.05)(D, F) * (D ** -0.5)),
            "w2": _w((lambda *s: _rng.normal(s) * 0.05)(F, D) * (F ** -0.5)),
        }
    _B_in = _B_setup()

    return {
        "A_x": _A_in["x"],
        "A_w_r": _A_in["w_r"],
        "A_w_i": _A_in["w_i"],
        "B_x": _B_in["x"],
        "B_w1": _B_in["w1"],
        "B_w2": _B_in["w2"],
        "gate_w": _w((lambda *s: _rng.normal(s) * 0.05)(512) * 16.0),
    }

def reference(A_x, A_w_r, A_w_i, B_x, B_w1, B_w2, gate_w):
    def _A_ref(x, w_r, w_i):
        B, S, D = x.shape
        X = (lambda x, axes=(-2,-1): jnp.fft.rfft2(x.astype(jnp.float32), axes=axes))(x, axes=(-2, -1))
        W = w_r + 1j * w_i
        X = X * W
        y = (lambda x, s, axes=(-2,-1): jnp.fft.irfft2(x, s=s, axes=axes).astype(jnp.bfloat16))(X, (S, D), axes=(-2, -1))
        return y

    def _B_ref(x, w1, w2):
        h = jnp.einsum("bsd,df->bsf", x, w1)
        h = _silu(h)
        out = jnp.einsum("bsf,fd->bsd", h, w2)
        return out

    x = A_x
    g = _sigmoid((x * gate_w).sum(-1, keepdims=True))
    a = _A_ref(x, A_w_r, A_w_i)
    b = _B_ref(x, B_w1, B_w2)
    return g * a + (1 - g) * b
```

```python
import numpy as np
import jax
import jax.numpy as jnp
import jax.experimental.pallas as pl
import jax.experimental.pallas.tpu as pltpu

S, D, F = 2048, 512, 1376
R, M = 16, 128
BF, F32 = jnp.bfloat16, jnp.float32


def _consts():
    m = np.arange(D)[:, None]
    k = np.arange(256)[None, :]
    ang = 2 * np.pi * ((m * k) % D) / D
    fd = np.zeros((D, 512))
    fd[:, :256] = np.cos(ang)
    fd[:, 256:512] = -np.sin(ang)
    c = np.full((256, 1), 2.0)
    c[0] = 1.0
    sc = 1.0 / (S * D)
    fi = np.zeros((512, D))
    fi[:256] = c * np.cos(ang.T) * sc
    fi[256:512] = -c * np.sin(ang.T) * sc
    k1 = np.arange(R)[:, None, None]
    k2 = np.arange(M)[None, :, None]
    n2 = np.arange(M)[None, None, :]
    a = -2 * np.pi * ((n2 * (k1 + R * k2)) % S) / S
    gr, gi = np.cos(a), np.sin(a)
    g = np.concatenate([np.concatenate([gr, -gi], 2), np.concatenate([gi, gr], 2)], 1)
    h = np.transpose(g, (0, 2, 1))
    cv = lambda t: np.asarray(t, np.float32).astype(BF)
    t = 2 * np.pi * np.arange(R)[:, None] * np.arange(M)[None, :] / S
    q = 2 * np.pi * np.arange(R)[:, None] * np.arange(M)[None, :] / R * (np.arange(M) < R)
    v = np.arange(M) < R
    cst = np.concatenate([np.cos(t), np.sin(t), np.cos(q) * v, np.sin(q) * v], 0).astype(np.float32)
    return cv(fd), cv(fi), cv(g), cv(h), cst


def _fft(xs, sign):
    n = len(xs)
    if n == 1:
        return xs
    ev, od = _fft(xs[0::2], sign), _fft(xs[1::2], sign)
    out = [None] * n
    for k in range(n // 2):
        (er, ei), (pr, pi) = ev[k], od[k]
        if k == 0:
            tr, ti = pr, pi
        elif 4 * k == n:
            if pi is None:
                out[k] = (er, sign * pr if ei is None else ei + sign * pr)
                out[k + n // 2] = (er, -sign * pr if ei is None else ei - sign * pr)
                continue
            tr, ti = (-pi, pr) if sign > 0 else (pi, -pr)
        else:
            c = float(np.cos(2 * np.pi * k / n))
            s = float(sign * np.sin(2 * np.pi * k / n))
            if pi is None:
                tr, ti = pr * c, pr * s
            elif 8 * k == n:
                tr, ti = ((pr - pi) * c, (pr + pi) * c) if sign > 0 else ((pr + pi) * c, (pi - pr) * c)
            elif 8 * k == 3 * n:
                tr, ti = ((pr + pi) * c, (pi - pr) * c) if sign > 0 else ((pr - pi) * c, (pr + pi) * c)
            else:
                tr, ti = pr * c - pi * s, pr * s + pi * c
        if ti is None:
            out[k], out[k + n // 2] = (er + tr, ei), (er - tr, ei)
        elif ei is None:
            out[k], out[k + n // 2] = (er + tr, ti), (er - tr, -ti)
        else:
            out[k], out[k + n // 2] = (er + tr, ei + ti), (er - tr, ei - ti)
    return out


def _kernel(x_h, wr_h, wi_h, w1_h, w2_h, gw_h, fd_h, fi_h, g_h, h_h, c_h, wn_h, o_h,
            x_v, wr_v, wi_v, c_v, wn_v, wrt_v, wit_v, w1_v, w2_v, gw_v, fd_v, fi_v, g_v, h_v,
            xs, ys, zs, b_v, gs, o_v, sems, osem):
    srcs = (x_h, fd_h, w1_h, w2_h, g_h, h_h, fi_h, gw_h, c_h, wn_h)
    dsts = (x_v, fd_v, w1_v, w2_v, g_v, h_v, fi_v, gw_v, c_v, wn_v)
    for a, b in ((wr_h, wrt_v), (wi_h, wit_v)):
        srcs += (a.at[0:256],)
        dsts += (b,)
    cps = [pltpu.make_async_copy(s, d, sems.at[i]) for i, (s, d) in enumerate(zip(srcs, dsts))]
    cps[0].start()
    cps[1].start()
    cps[7].start()
    cx, cfd, cw1, cw2, cg, ch, cfi, cgw, cc, cwn = cps[:10]
    dot = lambda a, b: jnp.dot(a, b, preferred_element_type=F32)

    def ffn(r0, n):
        h = jax.lax.dot_general(x_v[pl.ds(r0, n), :], w1_v[...], (((1,), (1,)), ((), ())),
                                preferred_element_type=F32)
        h = 0.5 * h
        h = h + h * jnp.tanh(h)
        b_v[pl.ds(r0, n), :] = dot(h.astype(BF), w2_v[...])

    cx.wait()
    cfd.wait()
    cgw.wait()
    for c in cps[2:7] + cps[8:]:
        c.start()

    def p1(i, _):
        r0 = pl.multiple_of(i * 512, 512)
        xs[pl.ds(r0, 512), :] = dot(x_v[pl.ds(r0, 512), :], fd_v[...])
        xb = x_v[pl.ds(r0, 512), :].astype(F32)
        gs[pl.ds(r0, 512), :] = jax.nn.sigmoid(jnp.sum(xb * gw_v[...].astype(F32), axis=-1, keepdims=True))
    for i in range(4):
        p1(i, None)
    cw1.wait()
    cw2.wait()

    NI = 4
    SL = M // NI
    FR = S // (2 * NI)

    def p2(i, _):
        ffn(pl.multiple_of(i * FR, FR), FR)
        for j in range(SL // 16):
            r = pl.multiple_of(i * SL + j * 16, 16)
            for t in range(2):
                if t < 2:
                    v = [(xs[pl.ds(n * M + r, 16), pl.ds(t * 128, 128)],
                          xs[pl.ds(n * M + r, 16), pl.ds(256 + t * 128, 128)]) for n in range(R)]
                else:
                    v = [(xs[pl.ds(n * M + r, 16), pl.ds(512, 128)], None) for n in range(R)]
                for k, (a, b) in enumerate(_fft(v, -1)):
                    ys[k, pl.ds(r, 16), pl.ds(t * 128, 128)] = a.astype(BF)
                    ys[k, pl.ds(M + r, 16), pl.ds(t * 128, 128)] = (jnp.zeros_like(a) if b is None else b).astype(BF)
    for i in range(NI):
        p2(i, None)
    cg.wait()
    for c in cps[10:]:
        c.wait()
    ch.wait()

    for a, b in ((wrt_v, wr_v), (wit_v, wi_v)):
        for t in range(2):
            b[t * S:(t + 1) * S, :] = a[t * 128:(t + 1) * 128, :].T
    wr32 = wr_v.bitcast(jnp.uint32)
    wi32 = wi_v.bitcast(jnp.uint32)
    cc.wait()
    cwn.wait()
    io = lambda sh, d: jax.lax.broadcasted_iota(jnp.int32, sh, d)
    alt = lambda sh: (1 - 2 * (io(sh, 1) & 1)).astype(F32)
    sel = lambda sh, n: jnp.where(io(sh, 0) == n, alt(sh), 0.0).astype(BF)
    tn = jnp.zeros((R, M), F32)
    for n in range(R):
        xb = x_v[n * M:(n + 1) * M, :].astype(F32)
        fo = (xb[:, :128] + xb[:, 128:256]) + (xb[:, 256:384] + xb[:, 384:])
        tn = tn + jax.lax.dot_general(sel((R, 128), n), fo.astype(BF), (((1,), (1,)), ((), ())),
                                      preferred_element_type=F32)
    tc, ts = c_v[0:16], c_v[16:32]
    qc, qs = c_v[32:48, 0:16].astype(BF), c_v[48:64, 0:16].astype(BF)
    tb = tn.astype(BF)
    ur, ui = dot(qc, tb), -dot(qs, tb)
    v = dot(jnp.concatenate([ur * tc + ui * ts, ui * tc - ur * ts], 1).astype(BF), h_v[0])
    vr, vi = v[:, :M], v[:, M:]
    nr, ni = wn_v[0:16].astype(F32), wn_v[16:32].astype(F32)
    v = dot(jnp.concatenate([vr * nr - vi * ni, vr * ni + vi * nr], 1).astype(BF), g_v[0])
    vr, vi = v[:, :M], v[:, M:]
    yn = dot(qc, (vr * tc - vi * ts).astype(BF)) - dot(qs, (vi * tc + vr * ts).astype(BF))
    ynt = (jnp.concatenate([yn, jnp.zeros((M - R, M), F32)], 0).T * (1.0 / (S * D)))

    def p3(kk, _):
        def ld(ref):
            a = [ref[pl.ds(t * (S // 2) + kk, M, stride=8), :] for t in range(2)]
            return jnp.concatenate(a, axis=1)
        pr, pi = ld(wr32), ld(wi32)
        for half in range(2):
            k = 2 * kk + half
            if half == 0:
                cv = lambda p: pltpu.bitcast(p << 16, F32)
            else:
                cv = lambda p: pltpu.bitcast(p & jnp.uint32(0xFFFF0000), F32)
            wr, wi = cv(pr), cv(pi)
            z = dot(g_v[k], ys[k])
            zr, zi = z[:M], z[M:]
            u = jnp.concatenate([zr * wr - zi * wi, zr * wi + zi * wr], axis=0).astype(BF)
            zs[k] = dot(h_v[k], u)
    for kk in range(R // 2):
        p3(kk, None)

    def p4(i, _):
        ffn(pl.multiple_of((NI + i) * FR, FR), FR)
        for j in range(SL // 16):
            r = pl.multiple_of(i * SL + j * 16, 16)
            for t in range(2):
                v = [(zs[k, pl.ds(r, 16), pl.ds(t * 128, 128)],
                      zs[k, pl.ds(M + r, 16), pl.ds(t * 128, 128)]) for k in range(R)]
                for n, (a, b) in enumerate(_fft(v, 1)):
                    if t < 2:
                        ys[n, pl.ds(r, 16), pl.ds(t * 128, 128)] = a.astype(BF)
                        ys[n, pl.ds(M + r, 16), pl.ds(t * 128, 128)] = b.astype(BF)
                    else:
                        ys[n, pl.ds(r, 16), pl.ds(256, 128)] = a.astype(BF)
    for i in range(NI):
        p4(i, None)
    cfi.wait()

    ocs = []
    for n in range(R):
        y = ys[n]
        lhs = jnp.concatenate([y[:M, :256], y[M:, :256]], axis=1)
        a = dot(lhs, fi_v[...]) + ynt[:, n:n + 1] * alt((1, D))
        g = gs[n * M:(n + 1) * M, :]
        b = b_v[n * M:(n + 1) * M, :]
        o_v[n * M:(n + 1) * M, :] = (b + g * (a - b)).astype(BF)
        if n % 4 == 3:
            q = n // 4
            c = pltpu.make_async_copy(o_v.at[pl.ds(q * 512, 512)], o_h.at[pl.ds(q * 512, 512)], osem.at[q])
            c.start()
            ocs.append(c)
    for c in ocs:
        c.wait()


@jax.jit
def pallas_gated_mix__spectral_gfnet__dense_activation_silu__prompt_kernel(
    A_x, A_w_r, A_w_i, B_x, B_w1, B_w2, gate_w,
):
    fd, fi, g, h, cst = _consts()
    wn = jnp.concatenate([A_w_r.T[256].reshape(M, R).T, A_w_i.T[256].reshape(M, R).T], 0)
    V = pltpu.VMEM
    out = pl.pallas_call(
        _kernel,
        out_shape=jax.ShapeDtypeStruct((S, D), BF),
        in_specs=[pl.BlockSpec(memory_space=pltpu.HBM)] * 12,
        out_specs=pl.BlockSpec(memory_space=pltpu.HBM),
        scratch_shapes=[
            V((S, D), BF), V((2 * S, 128), BF), V((2 * S, 128), BF), V((64, 128), F32), V((32, 128), BF), V((256, S), BF), V((256, S), BF), V((F, D), BF), V((F, D), BF), V((1, D), BF),
            V((D, 512), BF), V((512, D), BF), V((R, 256, 256), BF), V((R, 256, 256), BF),
            V((S, 512), F32), V((R, 256, 256), BF), V((R, 256, 256), F32), V((S, D), F32), V((S, 1), F32), V((S, D), BF),
            pltpu.SemaphoreType.DMA((14,)), pltpu.SemaphoreType.DMA((4,)),
        ],
        compiler_params=pltpu.CompilerParams(vmem_limit_bytes=100 * 1024 * 1024),
    )(A_x.reshape(S, D), A_w_r.T, A_w_i.T, B_w1.T, B_w2, gate_w.reshape(1, D), fd, fi, g, h, cst, wn)
    return out.reshape(1, S, D)
```
